```python
import os as _os
_os.environ.setdefault("JAX_PLATFORMS", "cpu")
import jax
import jax.numpy as jnp

def _softmax(x, axis=-1):
    return jax.nn.softmax(x, axis=axis)
def _gelu(x):
    return jax.nn.gelu(x, approximate=True)
def _silu(x):
    return jax.nn.silu(x)
def _sigmoid(x):
    return jax.nn.sigmoid(x)
def _layernorm(x, axis=-1, eps=1e-5):
    m = jnp.mean(x, axis=axis, keepdims=True)
    v = jnp.var(x, axis=axis, keepdims=True)
    return (x - m) / jnp.sqrt(v + eps)
def _scatter_add(tgt, idx, src, axis=0):
    return tgt.at[idx].add(src)
def _segment_sum(src, seg, n):
    return jax.ops.segment_sum(src, seg, n)
class _Rng:
    def __init__(self, key):
        self._k = key
    def _next(self):
        self._k, sub = jax.random.split(self._k)
        return sub
    def normal(self, shape):
        return jax.random.normal(self._next(), shape, dtype=jnp.bfloat16)
    def randint(self, lo, hi, shape):
        return jax.random.randint(self._next(), shape, lo, hi, dtype=jnp.int32)
    def uniform(self, shape, lo=0.0, hi=1.0):
        return jax.random.uniform(self._next(), shape, jnp.bfloat16, lo, hi)
    def permutation(self, n):
        return jax.random.permutation(self._next(), n)


kernel_name = 'concat_heads__gqa_block_cached__mha_block_cached__near_ridge'

def setup_inputs():
    _rng = _Rng(jax.random.key(int.from_bytes(__import__("os").urandom(4), "little")))
    _w = (lambda a: (lambda t: t.astype(jnp.bfloat16) if jnp.issubdtype(t.dtype, jnp.floating) else t)(jnp.asarray(a)))
    def _A_setup():
        B, Sq, D = 8, 96, 640
        Hq, Hkv, Sk, Dh = 32, 32, 512, 128
        assert Hq % Hkv == 0, (Hq, Hkv)
        return {
            "x": _w((lambda *s: _rng.normal(s) * 0.8)(B, Sq, D)),
            "k_cache": _w((lambda *s: _rng.normal(s) * 0.8)(B, Hkv, Sk, Dh)),
            "v_cache": _w((lambda *s: _rng.normal(s) * 0.05)(B, Hkv, Sk, Dh)),
            "wq": _w((lambda *s: _rng.normal(s) * 0.8)(D, Hq * Dh) * (D ** -0.5)),
            "wo": _w((lambda *s: _rng.normal(s) * 0.05)(Hq * Dh, D) * ((Hq * Dh) ** -0.5)),
        }
    _A_in = _A_setup()

    def _B_setup():
        B, Sq, D = 8, 96, 640
        H, Sk, Dh = 32, 512, 128
        return {
            "x": _w((lambda *s: _rng.normal(s) * 0.8)(B, Sq, D)),
            "k_cache": _w((lambda *s: _rng.normal(s) * 0.8)(B, H, Sk, Dh)),
            "v_cache": _w((lambda *s: _rng.normal(s) * 0.05)(B, H, Sk, Dh)),
            "wq": _w((lambda *s: _rng.normal(s) * 0.8)(D, H * Dh) * (D ** -0.5)),
            "wo": _w((lambda *s: _rng.normal(s) * 0.05)(H * Dh, D) * ((H * Dh) ** -0.5)),
        }
    _B_in = _B_setup()

    return {
        "A_x": _A_in["x"],
        "A_k_cache": _A_in["k_cache"],
        "A_v_cache": _A_in["v_cache"],
        "A_wq": _A_in["wq"],
        "A_wo": _A_in["wo"],
        "B_x": _B_in["x"],
        "B_k_cache": _B_in["k_cache"],
        "B_v_cache": _B_in["v_cache"],
        "B_wq": _B_in["wq"],
        "B_wo": _B_in["wo"],
    }

def reference(A_x, A_k_cache, A_v_cache, A_wq, A_wo, B_x, B_k_cache, B_v_cache, B_wq, B_wo):
    def _A_ref(x, k_cache, v_cache, wq, wo):
        B, Sq, D = x.shape
        Hq, Dh = 32, 128
        Hkv = k_cache.shape[1]
        rep = Hq // Hkv
        q = (lambda x, *d: x.transpose(*d))((x @ wq).reshape(B, Sq, Hq, Dh), 0, 2, 1, 3)
        k = jnp.repeat(k_cache, rep, axis=1)
        v = jnp.repeat(v_cache, rep, axis=1)
        scores = jnp.einsum("bhqd,bhkd->bhqk", q, k) * (Dh ** -0.5)
        p = _softmax(scores, axis=-1)
        o = jnp.einsum("bhqk,bhkd->bhqd", p, v)
        return (lambda x, *d: x.transpose(*d))(o, 0, 2, 1, 3).reshape(B, Sq, Hq * Dh) @ wo

    def _B_ref(x, k_cache, v_cache, wq, wo):
        B, Sq, D = x.shape
        H, Dh = 32, 128
        q = (lambda x, *d: x.transpose(*d))((x @ wq).reshape(B, Sq, H, Dh), 0, 2, 1, 3)
        scores = jnp.einsum("bhqd,bhkd->bhqk", q, k_cache) * (Dh ** -0.5)
        p = _softmax(scores, axis=-1)
        o = jnp.einsum("bhqk,bhkd->bhqd", p, v_cache)
        return (lambda x, *d: x.transpose(*d))(o, 0, 2, 1, 3).reshape(B, Sq, H * Dh) @ wo

    a = _A_ref(A_x, A_k_cache, A_v_cache, A_wq, A_wo)
    b = _B_ref(B_x, B_k_cache, B_v_cache, B_wq, B_wo)
    return jnp.concatenate([a, b], axis=-1)
```

```python
import numpy as np
import jax
import jax.numpy as jnp
from jax import lax
from jax.experimental import pallas as pl
from jax.experimental.pallas import tpu as pltpu

B, SQ, D, H, SK, DH = 8, 96, 640, 32, 512, 128
G = 4
NG = H // G
UB = NG * B
NU = 2 * UB
QSCALE = float(DH ** -0.5 * np.log2(np.e))
NT = (((1,), (1,)), ((), ()))
F32, BF16, U32 = jnp.float32, jnp.bfloat16, jnp.uint32

def make(NB=8, NW=3, dma=True, flags=None, order="K0 Q V0 K1 O01 V1 K2 O23 V2 K3 O4 V3", u32=True):
    def kern(ax, ak, av, awq, awo, bx, bk, bv, bwq, bwo, out, xb, kb, vb, wqb, wob, qb, ob, acc, res, sem, wsem, xsem, osem):
        def kv_copies(k, v, u, slot):
            b, hg = u % B, u // B
            return [pltpu.make_async_copy(k.at[b, pl.ds(hg * G, G)], kb.at[slot], sem.at[0, slot]),
                    pltpu.make_async_copy(v.at[b, pl.ds(hg * G, G)], vb.at[slot], sem.at[1, slot])]
        def wq_copy(wq, hg, slot):
            c = pl.multiple_of(hg * (G * DH), G * DH)
            return pltpu.make_async_copy(wq.at[:, pl.ds(c, G * DH)], wqb.at[slot], wsem.at[0, slot])
        def wo_copy(wo, hg, slot):
            c = pl.multiple_of(hg * (G * DH), G * DH)
            return pltpu.make_async_copy(wo.at[pl.ds(c, G * DH), :], wob.at[slot], wsem.at[1, slot])
        def two(i, n, fa, fb):
            pl.when(i < n)(lambda: fa(i))
            pl.when(jnp.logical_and(i >= n, i < 2 * n))(lambda: fb(i - n))
        def start_kv(u):
            def go(k, v):
                def f(i):
                    for j, c in enumerate(kv_copies(k, v, i, u % NB)): c.start(priority=j)
                return f
            two(u, UB, go(ak, av), go(bk, bv))
        def start_wq(w): two(w, NG, lambda i: wq_copy(awq, i, w % NW).start(), lambda i: wq_copy(bwq, i, w % NW).start())
        def start_wo(w): two(w, NG, lambda i: wo_copy(awo, i, w % NW).start(priority=1), lambda i: wo_copy(bwo, i, w % NW).start(priority=1))
        xc = [pltpu.make_async_copy(ax, xb.at[pl.ds(0, B)], xsem.at[0]), pltpu.make_async_copy(bx, xb.at[pl.ds(B, B)], xsem.at[1])]
        def out_copy(br, b): return pltpu.make_async_copy(res.at[br, b], out.at[b, :, pl.ds(br * D, D)], osem.at[br, b])

        def ld(ref, *idx):
            if u32: return pltpu.bitcast(ref.bitcast(U32)[idx], BF16)
            return ref[idx]
        def qproj(u):
            q = jnp.dot(xb[(u // UB) * B + u % B], wqb[(u // B) % NW], preferred_element_type=F32)
            qb[u % 2] = pltpu.bitcast((q * QSCALE).astype(BF16), U32)
        def oproj(u, n0, n1):
            cs = slice(n0 * 128, n1 * 128)
            r = jnp.dot(pltpu.bitcast(ob[u % 2], BF16), wob[(u // B) % NW, :, cs], preferred_element_type=F32)
            acc[(u // UB) * B + u % B, :, cs] += r
        def scores(u, g):
            q = pltpu.bitcast(qb[u % 2, :, g * DH:(g + 1) * DH], BF16)
            s = lax.dot_general(q, ld(kb, u % NB, g), NT, preferred_element_type=F32)
            p = jnp.exp2(s - jnp.max(s, axis=-1, keepdims=True))
            l = jnp.sum(p, axis=-1, keepdims=True)
            r = pl.reciprocal(l, approx=True)
            return p.astype(BF16), r * (2.0 - l * r)
        def pv(u, g, p, r):
            o = jnp.dot(p, ld(vb, u % NB, g), preferred_element_type=F32)
            ob[u % 2, :, g * DH:(g + 1) * DH] = pltpu.bitcast((o * r).astype(BF16), U32)
        def unit(u, un, up):
            st = {}
            for op in order.split():
                if op[0] == "K": st[op[1]] = scores(u, int(op[1]))
                elif op[0] == "V": pv(u, int(op[1]), *st[op[1]])
                elif op[0] == "Q":
                    if un is not None: qproj(un)
                elif up is not None: oproj(up, int(op[1]), int(op[-1]) + 1)

        z = jnp.int32(0)
        xc[0].start(); start_wq(z); start_kv(z); start_wo(z)
        for t in range(1, NB): start_kv(z + t)
        start_wq(z + 1); start_wo(z + 1)
        xc[1].start()
        acc[...] = jnp.zeros_like(acc)
        ob[1] = jnp.zeros(ob.shape[1:], U32)
        xc[0].wait(); wq_copy(awq, 0, 0).wait()
        qproj(z)
        wo_copy(awo, 0, 0).wait()
        if not dma:
            for t in range(NB):
                for cp in kv_copies(ak, av, 0, t): cp.wait()
        def finish(br, b):
            res[br, b] = acc[br * B + b].astype(BF16)
        def body(u, c):
            w = u // B
            @pl.when(jnp.logical_and(u % B == B - 1, u < NU - 1))
            def _(): wq_copy(awq, 0, (w + 1) % NW).wait()
            @pl.when(jnp.logical_and(u % B == 1, u > 1))
            def _(): wo_copy(awo, 0, w % NW).wait()
            @pl.when(u == UB - 1)
            def _(): xc[1].wait()
            if dma:
                for cp in kv_copies(ak, av, 0, u % NB): cp.wait()
            unit(u, jnp.where(u == NU - 1, u - 1, u + 1), jnp.where(u == 0, 1, u - 1))
            if dma: start_kv(u + NB)
            @pl.when(u % B == 1)
            def _(): start_wq(w + 2)
            @pl.when(u % B == 4)
            def _(): start_wo(w + 2)
            @pl.when(u == UB)
            def _():
                for b in range(B): finish(0, b)
            @pl.when(u == NU - NB)
            def _():
                for b in range(B): out_copy(0, b).start()
            @pl.when(u > NU - B)
            def _():
                finish(1, u - 1 - (NU - B)); out_copy(1, u - 1 - (NU - B)).start()
            return c
        lax.fori_loop(0, NU, body, 0)
        oproj(z + NU - 1, 0, 5)
        finish(1, B - 1); out_copy(1, B - 1).start()
        for br in range(2):
            for b in range(B): out_copy(br, b).wait()
    @jax.jit
    def f(ax, ak, av, awq, awo, bx, bk, bv, bwq, bwo):
        return pl.pallas_call(kern, out_shape=jax.ShapeDtypeStruct((B, SQ, 2 * D), BF16),
            in_specs=[pl.BlockSpec(memory_space=pl.ANY)] * 10, out_specs=pl.BlockSpec(memory_space=pl.ANY),
            scratch_shapes=[pltpu.VMEM((2 * B, SQ, D), BF16), pltpu.VMEM((NB, G, SK, DH), BF16), pltpu.VMEM((NB, G, SK, DH), BF16),
                pltpu.VMEM((NW, D, G * DH), BF16), pltpu.VMEM((NW, G * DH, D), BF16),
                pltpu.VMEM((2, SQ // 2, G * DH), U32), pltpu.VMEM((2, SQ // 2, G * DH), U32),
                pltpu.VMEM((2 * B, SQ, D), F32), pltpu.VMEM((2, B, SQ, D), BF16),
                pltpu.SemaphoreType.DMA((2, NB)), pltpu.SemaphoreType.DMA((2, NW)), pltpu.SemaphoreType.DMA((2,)), pltpu.SemaphoreType.DMA((2, B))],
            compiler_params=pltpu.CompilerParams(vmem_limit_bytes=100 << 20, flags=flags),
        )(ax, ak, av, awq, awo, bx, bk, bv, bwq, bwo)
    return f


_impl = make()

@jax.jit
def pallas_concat_heads__gqa_block_cached__mha_block_cached__near_ridge_kernel(A_x, A_k_cache, A_v_cache, A_wq, A_wo, B_x, B_k_cache, B_v_cache, B_wq, B_wo):
    return _impl(A_x, A_k_cache, A_v_cache, A_wq, A_wo, B_x, B_k_cache, B_v_cache, B_wq, B_wo)
```

```python
import numpy as np
import jax
import jax.numpy as jnp
from jax import lax
from jax.experimental import pallas as pl
from jax.experimental.pallas import tpu as pltpu

B, SQ, D, H, SK, DH = 8, 96, 640, 32, 512, 128
G = 4
GD = G * DH
NG = H // G
UB = NG * B
NU = 2 * UB
QSCALE = float(DH ** -0.5 * np.log2(np.e))
NT = (((1,), (1,)), ((), ()))
F32, BF16, U32 = jnp.float32, jnp.bfloat16, jnp.uint32
PR = 128
ORD = "D K0 D Q D V0 K1 D O01 D V1 K2 D O23 D V2 K3 D O4 V3"
TORD = "D K0 D K1 D O01 D V0 K2 D O23 D V1 K3 D O4 D V2 V3"

def make(L=3, NB=4, dma=True, flags=None, order=ORD, tord=TORD, wpos=(3, 7, 11, 15), xat=1, wr=16, wsched=None, wo0=1, swap=0, xsplit=1):
    NW = 4
    wsched = wsched or {(6, 0): ((0, 1), (2, 3), (4,)), (7, 0): ((5,),)}
    def kern(ax, ak, av, awq, awo, bx, bk, bv, bwq, bwo, out, xb, kb, vb, wqb, wob, qb, ob, acc, res, sem, wsem, xsem, osem):
        def head(w, g): return (w & (NG - 1)) + g * NG
        def kv_piece(j, br, v, g, r):
            src, dst = ((ak, av), (bk, bv))[br][j], (kb, vb)[j]
            return pltpu.make_async_copy(src.at[v & (B - 1), head(v >> 3, g), pl.ds(r, PR)], dst.at[v % NB, g, pl.ds(r, PR)], sem.at[j, v % NB])
        def wq_piece(br, w, g, r0, n):
            c = pl.multiple_of(head(w, g) * DH, DH)
            return pltpu.make_async_copy((awq, bwq)[br].at[pl.ds(r0, n), pl.ds(c, DH)], wqb.at[w % NW, g, pl.ds(r0, n)], wsem.at[0, w % NW])
        def wo_piece(br, w, i):
            r = pl.multiple_of(i * 16, 16)
            c = pl.multiple_of(head(w, i >> 3) * DH + (r & (DH - 1)), 16)
            return pltpu.make_async_copy((awo, bwo)[br].at[pl.ds(c, 16)], wob.at[w % NW, pl.ds(r, 16)], wsem.at[1, w % NW])
        def both(i, n): return (i < n, jnp.logical_and(i >= n, i < 2 * n))
        def w_items(wq, wo, b, n):
            r0 = pl.multiple_of(b * (D // B), 16)
            return [(both(wq, NG), lambda br: wq_piece(br, wq, n, r0, D // B).start(priority=swap)),
                    (both(wo, NG), lambda br: wo_piece(br, wo, b * 4 + n).start(priority=1 - swap))]
        def issue_list(v, weights=True):
            lst, c = [], both(v, UB)
            for i in range(16):
                lst.append((c, lambda br, i=i: [kv_piece(j, br, v, i & 3, (i >> 2) * PR).start(priority=j) for j in range(2)]))
                if weights:
                    for n, pos in enumerate(wpos):
                        if pos == i: lst += w_items((v >> 3) + 2, (v >> 3) + 1, v & (B - 1), n)
            return lst
        def run(items, brs):
            for cond, go in items:
                for br in brs:
                    @pl.when(cond[br])
                    def _(): go(br)
        def wait_all(buf, s): pltpu.make_async_copy(buf, buf, s).wait()
        def wait_kv(u):
            for j, dst in enumerate((kb, vb)): wait_all(dst.at[u % NB], sem.at[j, u % NB])
        def wait_wq(w): wait_all(wqb.at[w % NW], wsem.at[0, w % NW])
        def wait_wo(w): wait_all(wob.at[w % NW], wsem.at[1, w % NW])
        def x_piece(br, b, r, n): return pltpu.make_async_copy((ax, bx)[br].at[b, pl.ds(r, n)], xb.at[br * B + b, pl.ds(r, n)], xsem.at[br])
        def wait_x(br): wait_all(xb.at[pl.ds(br * B, B)], xsem.at[br])
        def write(bs):
            for i, (r, b) in enumerate((r, b) for r in range(0, SQ, wr) for b in bs):
                pltpu.make_async_copy(res.at[b, pl.ds(r, wr)], out.at[b, pl.ds(r, wr)], osem.at[0]).start(priority=i % 2)

        def ld(ref, *idx): return pltpu.bitcast(ref.bitcast(U32)[idx], BF16)
        def row(u): return ((u >> 6) << 3) | (u & (B - 1))
        def qproj(u):
            w = jnp.concatenate([ld(wqb, (u >> 3) % NW, g) for g in range(G)], axis=1)
            q = (jnp.dot(xb[row(u)], w, preferred_element_type=F32) * QSCALE).astype(BF16)
            for g in range(G): qb[u & 15, g] = q[:, g * DH:(g + 1) * DH]
        def oproj(u, n0, n1, last):
            cs = slice(n0 * 128, n1 * 128)
            o = jnp.concatenate([ld(ob, u & 1, g) for g in range(G)], axis=1)
            r = acc[row(u), :, cs] + jnp.dot(o, wob[(u >> 3) % NW, :, cs], preferred_element_type=F32)
            acc[row(u), :, cs] = r
            if last: res[u & (B - 1), :, D + n0 * 128:D + n1 * 128] = r.astype(BF16)
        def scores(u, g):
            s = lax.dot_general(ld(qb, u & 15, g), ld(kb, u % NB, g), NT, preferred_element_type=F32)
            p = jnp.exp2(s - jnp.max(s, axis=-1, keepdims=True))
            l = jnp.sum(p, axis=-1, keepdims=True)
            r = pl.reciprocal(l, approx=True)
            return p.astype(BF16), r * (2.0 - l * r)
        def pv(u, g, p, r):
            o = jnp.dot(p, ld(vb, u % NB, g), preferred_element_type=F32)
            ob[u & 1, g] = (o * r).astype(BF16)
        def unit(u, up, ops, items, brs, last):
            st = {}
            ops = ops.split()
            nd, di = ops.count("D"), 0
            for op in ops:
                if op == "D":
                    if dma: run(items[len(items) * di // nd:len(items) * (di + 1) // nd], brs)
                    if last:
                        for (t, d), bs in wsched.items():
                            if d == di:
                                for bb in bs: pl.when(u == NU - B + t)(lambda bb=bb: write(bb))
                    di += 1
                elif op[0] == "K": st[op[1]] = scores(u, int(op[1]))
                elif op[0] == "V": pv(u, int(op[1]), *st[op[1]])
                elif op[0] == "Q": qproj(u + B)
                else: oproj(up, int(op[1]), int(op[-1]) + 1, last)

        z = jnp.int32(0)
        for i in range(20):
            wq_piece(0, z, i % 4, (i // 4) * 128, 128).start(priority=0)
            if i < B: x_piece(0, i, 0, SQ).start(priority=1)
        @pl.loop(0, L - 1)
        def _(t):
            for it in issue_list(t): it[1](0)
            @pl.when(t == 0)
            def _():
                @pl.loop(0, 2 * B)
                def _(i): acc[i] = jnp.zeros((SQ, D), F32)
                ob[1] = jnp.zeros(ob.shape[1:], BF16)
        wait_x(0); wait_wq(z)
        @pl.loop(0, B)
        def _(b):
            for n in range(4):
                for it in w_items(z + 1, z, b, n): it[1](0)
                if n % 2 == 0:
                    i = b * 2 + n // 2
                    for j in range(2): kv_piece(j, 0, z + L - 1, i & 3, pl.multiple_of((i >> 2) * PR, PR)).start(priority=j)
            qproj(b)
        for n in range(4):
            for it in w_items(z + 2, z + 1, z + L - 1, n): it[1](0)
        if wo0: wait_wo(z)
        if not dma:
            for t in range(L): wait_kv(z + t)
            wait_wq(z + 1)
            wait_all(wqb.at[2, :, pl.ds(0, L * 80)], wsem.at[0, 2]); wait_all(wob.at[1, pl.ds(0, L * 64)], wsem.at[1, 1])
        @pl.loop(0, NU - B)
        def _(u):
            if dma:
                pl.when(u & (B - 1) == 0)(lambda: wait_wq((u >> 3) + 1))
                pl.when(jnp.logical_and(u & (B - 1) == 1, u > B))(lambda: wait_wo(u >> 3))
                wait_kv(u)
            pl.when(u == UB - B)(lambda: wait_x(1))
            if xsplit == 1: pl.when((u >> 3) == xat)(lambda: x_piece(1, u & (B - 1), 0, SQ).start())
            else: pl.when(u < 48)(lambda: x_piece(1, u & (B - 1), pl.multiple_of((u >> 3) * 16, 16), 16).start(priority=xsplit - 2))
            unit(u, jnp.where(u == 0, 1, u - 1), order, issue_list(u + L), (0, 1), False)
        if dma: wait_wo(z + 2 * NG - 1)
        @pl.loop(0, B)
        def _(b):
            u = NU - B + b
            if dma: wait_kv(u)
            res[b, :, :D] = acc[b].astype(BF16)
            unit(u, u - 1, tord, issue_list(u + L, False), (1,), True)
        done = [b for bs in wsched.values() for bb in bs for b in bb]
        write([b for b in range(B - 1) if b not in done])
        oproj(z + NU - 1, 0, 5, True)
        write([B - 1])
        wait_all(res, osem.at[0])
    @jax.jit
    def f(ax, ak, av, awq, awo, bx, bk, bv, bwq, bwo):
        return pl.pallas_call(kern, out_shape=jax.ShapeDtypeStruct((B, SQ, 2 * D), BF16),
            in_specs=[pl.BlockSpec(memory_space=pl.ANY)] * 10, out_specs=pl.BlockSpec(memory_space=pl.ANY),
            scratch_shapes=[pltpu.VMEM((2 * B, SQ, D), BF16), pltpu.VMEM((NB, G, SK, DH), BF16), pltpu.VMEM((NB, G, SK, DH), BF16),
                pltpu.VMEM((NW, G, D, DH), BF16), pltpu.VMEM((NW, GD, D), BF16),
                pltpu.VMEM((2 * B, G, SQ, DH), BF16), pltpu.VMEM((2, G, SQ, DH), BF16),
                pltpu.VMEM((2 * B, SQ, D), F32), pltpu.VMEM((B, SQ, 2 * D), BF16),
                pltpu.SemaphoreType.DMA((2, NB)), pltpu.SemaphoreType.DMA((2, NW)), pltpu.SemaphoreType.DMA((2,)), pltpu.SemaphoreType.DMA((1,))],
            compiler_params=pltpu.CompilerParams(vmem_limit_bytes=64 << 20, flags=flags, disable_bounds_checks=True),
        )(ax, ak, av, awq, awo, bx, bk, bv, bwq, bwo)
    return f


_impl = make(xsplit=2)

@jax.jit
def pallas_concat_heads__gqa_block_cached__mha_block_cached__near_ridge_kernel(A_x, A_k_cache, A_v_cache, A_wq, A_wo, B_x, B_k_cache, B_v_cache, B_wq, B_wo):
    return _impl(A_x, A_k_cache, A_v_cache, A_wq, A_wo, B_x, B_k_cache, B_v_cache, B_wq, B_wo)
```

```python
import jax
import jax.numpy as jnp
import numpy as np
from jax import lax
import jax.experimental.pallas as pl
import jax.experimental.pallas.tpu as pltpu

B, SQ, D = 8, 96, 640
H, SK, DH = 32, 512, 128

G = 4
NG = H // G
UNITS_PER_BRANCH = NG * B
UNITS = 2 * UNITS_PER_BRANCH

AHEAD = 3
SLOTS = 4
KV_ROWS = 128
WQ_ROWS = 40
WO_ROWS = 16
X_ROWS = 32
OUT_ROWS = 16
KV_PAIRS = G * SK // KV_ROWS
WQ_PAIRS = G * D // (2 * B * WQ_ROWS)
WO_PAIRS = G * DH // (2 * B * WO_ROWS)
X_PAIRS = B * SQ // (2 * X_ROWS)
TILES = D // 128

Q_SCALE = float(DH ** -0.5 * np.log2(np.e))

MAIN_STARTS = dict(
    qk=("qc", "c", "c", "cc"),
    q_proj=("qc", "c", "c", "c", "qc"),
    pv=("c", "c", "c", "qc"),
    out_proj=("oc", "", "oc", "", ""),
)
LAST_GROUP_STARTS = dict(
    qk=("c", "c", "cc", "cc"),
    pv=("cc", "cc", "cc", "cccc"),
    out_proj=("",) * TILES,
)

F32, BF16 = jnp.float32, jnp.bfloat16


def _branch(u):
    return u >> 6


def _group(u):
    return u >> 3


def _batch(u):
    return u & (B - 1)


def _head(u, g):
    return (_group(u) & (NG - 1)) + g * NG


def _slot(i):
    return i & (SLOTS - 1)


def _rows(start, size):
    if not isinstance(start, int):
        start = pl.multiple_of(start, size)
    return pl.ds(start, size)


def _wait_filled(buf, sem):
    pltpu.make_async_copy(buf, buf, sem).wait()


def _pipeline(x_hbm, k_hbm, v_hbm, wq_hbm, wo_hbm, out_hbm,
              x_buf, k_buf, v_buf, wq_buf, wo_buf, q_buf, acc, res, out_sem,
              kv_sem, wq_sem, wo_sem, x_sem):
    def start_kv(br, u, i):
        g, rows = i & (G - 1), _rows((i >> 2) * KV_ROWS, KV_ROWS)
        for j, (src, dst) in enumerate(((k_hbm[br], k_buf), (v_hbm[br], v_buf))):
            pltpu.make_async_copy(
                src.at[_batch(u), _head(u, g), rows],
                dst.at[_slot(u), g, rows],
                kv_sem.at[j, _slot(u)],
            ).start(priority=j)

    def start_wq(br, u, i):
        slot = _slot(_group(u))
        rows = pl.ds(pl.multiple_of(_batch(u) * (D // B) + (i >> 1) * WQ_ROWS, 8), WQ_ROWS)
        for j in range(2):
            g = 2 * (i & 1) + j
            pltpu.make_async_copy(
                wq_hbm[br].at[rows, _rows(_head(u, g) * DH, DH)],
                wq_buf.at[slot, g, rows],
                wq_sem.at[slot],
            ).start(priority=j)

    def start_wo(br, u, i):
        slot = _slot(_group(u))
        for j in range(2):
            g = 2 * i + j
            pltpu.make_async_copy(
                wo_hbm[br].at[_rows(_head(u, g) * DH + _batch(u) * WO_ROWS, WO_ROWS)],
                wo_buf.at[slot, _rows(g * DH + _batch(u) * WO_ROWS, WO_ROWS)],
                wo_sem.at[slot],
            ).start(priority=j)

    def start_x(br, i):
        rows = _rows((i >> 2) * X_ROWS, X_ROWS)
        for j in range(2):
            b = (i & 3) + 4 * j
            pltpu.make_async_copy(
                x_hbm[br].at[b, rows], x_buf.at[br, b, rows], x_sem.at[br]
            ).start(priority=j)

    def start_out(batches):
        pieces = [(b, pl.ds(r, OUT_ROWS)) for r in range(0, SQ, OUT_ROWS) for b in batches]
        for i, idx in enumerate(pieces):
            pltpu.make_async_copy(res.at[idx], out_hbm.at[idx], out_sem).start(priority=i % 2)

    def wait_kv(u):
        for j, buf in enumerate((k_buf, v_buf)):
            _wait_filled(buf.at[_slot(u)], kv_sem.at[j, _slot(u)])

    def wait_weights(buf, sem, u):
        _wait_filled(buf.at[_slot(_group(u))], sem.at[_slot(_group(u))])

    def q_proj(u, after_tile):
        w = []
        for t in range(TILES):
            w.append(jnp.concatenate(
                [wq_buf[_slot(_group(u)), g, t * 128:(t + 1) * 128] for g in range(G)], axis=1))
            after_tile(t)
        q = jnp.dot(x_buf[_branch(u), _batch(u)], jnp.concatenate(w, axis=0),
                    preferred_element_type=F32)
        q = (q * Q_SCALE).astype(BF16)
        for g in range(G):
            q_buf[u & (2 * B - 1), g] = q[:, g * DH:(g + 1) * DH]

    def unit(u, starts, branches):
        started = dict(c=0, q=0, o=0)
        streams = dict(c=(start_kv, u + AHEAD),
                       q=(start_wq, u + AHEAD + 2 * B),
                       o=(start_wo, u + AHEAD + B))

        def start(kinds):
            for kind in kinds:
                fn, target = streams[kind]
                for br in branches:
                    pl.when(_branch(target) == br)(lambda: fn(br, target, started[kind]))
                started[kind] += 1

        probs = []
        for g in range(G):
            s = lax.dot_general(q_buf[u & (2 * B - 1), g], k_buf[_slot(u), g],
                                (((1,), (1,)), ((), ())), preferred_element_type=F32)
            p = jnp.exp2(s - jnp.max(s, axis=-1, keepdims=True))
            probs.append((p.astype(BF16), 1.0 / jnp.sum(p, axis=-1, keepdims=True)))
            start(starts["qk"][g])
        if "q_proj" in starts:
            q_proj(u + B, lambda t: start(starts["q_proj"][t]))
        heads = []
        for g, (p, inv_sum) in enumerate(probs):
            o = jnp.dot(p, v_buf[_slot(u), g], preferred_element_type=F32)
            heads.append((o * inv_sum).astype(BF16))
            start(starts["pv"][g])
        w = []
        for t in range(TILES):
            w.append(wo_buf[_slot(_group(u)), :, t * 128:(t + 1) * 128])
            start(starts["out_proj"][t])
        assert started["c"] == KV_PAIRS
        assert (started["q"], started["o"]) in ((0, 0), (WQ_PAIRS, WO_PAIRS))
        return acc[_branch(u), _batch(u)] + jnp.dot(
            jnp.concatenate(heads, axis=1), jnp.concatenate(w, axis=1),
            preferred_element_type=F32)

    @pl.loop(0, X_PAIRS)
    def _(i):
        start_x(0, i)

    @pl.loop(0, B)
    def _(b):
        for i in range(WQ_PAIRS):
            start_wq(0, b, i)

    @pl.loop(0, B)
    def _(b):
        for i in range(2):
            start_kv(0, 0, 2 * b + i)
            start_wo(0, b, i)
            start_wq(0, B + b, i)
            start_wq(0, B + b, 2 + i)
            acc[i, b] = jnp.zeros((SQ, D), F32)

    @pl.loop(0, WQ_PAIRS)
    def _(i):
        start_wq(0, 2 * B, i)
        pl.when(i < WO_PAIRS)(lambda: start_wo(0, B, i))

    _wait_filled(x_buf.at[0], x_sem.at[0])
    wait_weights(wq_buf, wq_sem, 0)

    @pl.loop(0, B)
    def _(b):
        u, i = 1 + (b >> 2), b & 3
        for g in range(G):
            start_kv(0, u, G * i + g)
        start_wq(0, u + 2 * B, i)
        pl.when(i < WO_PAIRS)(lambda: start_wo(0, u + B, i))
        q_proj(b, lambda t: None)

    @pl.loop(0, UNITS - B)
    def _(u):
        @pl.when(_batch(u) == 0)
        def _():
            wait_weights(wo_buf, wo_sem, u)
            wait_weights(wq_buf, wq_sem, u + B)

        wait_kv(u)
        pl.when(u == UNITS_PER_BRANCH - B)(lambda: _wait_filled(x_buf.at[1], x_sem.at[1]))
        pl.when(u < X_PAIRS)(lambda: start_x(1, u))
        acc[_branch(u), _batch(u)] = unit(u, MAIN_STARTS, (0, 1))

    wait_weights(wo_buf, wo_sem, UNITS - B)

    @pl.loop(0, B)
    def _(b):
        u = UNITS - B + b
        wait_kv(u)
        res[b, :, :D] = acc[0, b].astype(BF16)
        pl.when(b == B - 2)(lambda: start_out(range(B - 2)))
        res[b, :, D:] = unit(u, LAST_GROUP_STARTS, (1,)).astype(BF16)
        pl.when(b == B - 2)(lambda: start_out([B - 2]))

    start_out([B - 1])


def _kernel(ax, ak, av, awq, awo, bx, bk, bv, bwq, bwo, out_hbm, *scratch):
    res, out_sem = scratch[-2:]
    pl.run_scoped(
        lambda *sems: _pipeline((ax, bx), (ak, bk), (av, bv), (awq, bwq), (awo, bwo),
                                out_hbm, *scratch, *sems),
        pltpu.SemaphoreType.DMA((2, SLOTS)),
        pltpu.SemaphoreType.DMA((SLOTS,)),
        pltpu.SemaphoreType.DMA((SLOTS,)),
        pltpu.SemaphoreType.DMA((2,)),
    )
    pltpu.make_async_copy(res, out_hbm, out_sem).wait()


@jax.jit
def pallas_concat_heads__gqa_block_cached__mha_block_cached__near_ridge_kernel(
    A_x: jax.Array,
    A_k_cache: jax.Array,
    A_v_cache: jax.Array,
    A_wq: jax.Array,
    A_wo: jax.Array,
    B_x: jax.Array,
    B_k_cache: jax.Array,
    B_v_cache: jax.Array,
    B_wq: jax.Array,
    B_wo: jax.Array,
):
    args = (A_x, A_k_cache, A_v_cache, A_wq, A_wo, B_x, B_k_cache, B_v_cache, B_wq, B_wo)
    shapes = ((B, SQ, D), (B, H, SK, DH), (B, H, SK, DH), (D, H * DH), (H * DH, D)) * 2
    assert all(a.shape == s and a.dtype == BF16 for a, s in zip(args, shapes))

    return pl.pallas_call(
        _kernel,
        out_shape=jax.ShapeDtypeStruct((B, SQ, 2 * D), BF16),
        in_specs=[pl.BlockSpec(memory_space=pl.ANY)] * len(args),
        out_specs=pl.BlockSpec(memory_space=pl.ANY),
        scratch_shapes=[
            pltpu.VMEM((2, B, SQ, D), BF16),
            pltpu.VMEM((SLOTS, G, SK, DH), BF16),
            pltpu.VMEM((SLOTS, G, SK, DH), BF16),
            pltpu.VMEM((SLOTS, G, D, DH), BF16),
            pltpu.VMEM((SLOTS, G * DH, D), BF16),
            pltpu.VMEM((2 * B, G, SQ, DH), BF16),
            pltpu.VMEM((2, B, SQ, D), F32),
            pltpu.VMEM((B, SQ, 2 * D), BF16),
            pltpu.SemaphoreType.DMA(()),
        ],
        compiler_params=pltpu.CompilerParams(
            vmem_limit_bytes=64 * 1024 * 1024,
            disable_bounds_checks=True,
        ),
    )(*args)
```

```python
import jax
import jax.numpy as jnp
import numpy as np
from jax import lax
import jax.experimental.pallas as pl
import jax.experimental.pallas.tpu as pltpu

B, SQ, D = 8, 96, 640
H, SK, DH = 32, 512, 128

G = 4
NG = H // G
UNITS_PER_BRANCH = NG * B
UNITS = 2 * UNITS_PER_BRANCH

AHEAD = 3
SLOTS = 4
KV_ROWS = 128
WQ_PARTS = ((0, 48), (48, 32))
WO_ROWS = 16
X_ROWS = 16
OUT_ROWS = 16
KV_PAIRS = G * SK // KV_ROWS
WQ_PAIRS = G // 2 * len(WQ_PARTS)
WO_PAIRS = G * DH // (2 * B * WO_ROWS)
X_PAIRS = B * SQ // (2 * X_ROWS)
TILES = D // 128

Q_SCALE = float(DH ** -0.5 * np.log2(np.e))

K_ORDER = (14, 0, 3, 1, 10, 6, 4, 5, 8, 11, 9, 7, 2, 12, 15, 13)
V_ORDER = (1, 3, 0, 2, 9, 5, 11, 4, 7, 6, 8, 10, 15, 13, 12, 14)
assert sorted(K_ORDER) == sorted(V_ORDER) == list(range(KV_PAIRS))

MAIN_STARTS = dict(
    qk=("qc", "c", "c", "cc"),
    q_proj=("qc", "c", "c", "c", "qc"),
    pv=("c", "c", "c", "qc"),
    out_proj=("oc", "", "oc", "", ""),
)
LAST_GROUP_STARTS = dict(
    qk=("c", "c", "cc", "cc"),
    pv=("cc", "cc", "cc", "cccc"),
    out_proj=("",) * TILES,
)

F32, BF16 = jnp.float32, jnp.bfloat16


def _branch(u):
    return u >> 6


def _group(u):
    return u >> 3


def _batch(u):
    return u & (B - 1)


def _head(u, g):
    return (_group(u) & (NG - 1)) + g * NG


def _slot(i):
    return i & (SLOTS - 1)


def _rows(start, size, align=None):
    if not isinstance(start, int):
        start = pl.multiple_of(start, align or size)
    return pl.ds(start, size)


def _wait_filled(buf, sem):
    pltpu.make_async_copy(buf, buf, sem).wait()


def _pipeline(x_hbm, k_hbm, v_hbm, wq_hbm, wo_hbm, out_hbm,
              x_buf, k_buf, v_buf, wq_buf, wo_buf, q_buf, acc, res, out_sem,
              kv_sem, wq_sem, wo_sem, x_sem):
    def start_kv(br, u, pieces):
        for j, (src, dst) in enumerate(((k_hbm[br], k_buf), (v_hbm[br], v_buf))):
            g, rows = pieces[j] & (G - 1), _rows((pieces[j] >> 2) * KV_ROWS, KV_ROWS)
            pltpu.make_async_copy(
                src.at[_batch(u), _head(u, g), rows],
                dst.at[_slot(u), g, rows],
                kv_sem.at[j, _slot(u)],
            ).start(priority=j)

    def start_wq(br, u, i, part=(0, D // B)):
        slot = _slot(_group(u))
        rows = _rows(_batch(u) * (D // B) + part[0], part[1], align=16)
        for j in range(2):
            g = 2 * i + j
            pltpu.make_async_copy(
                wq_hbm[br].at[rows, _rows(_head(u, g) * DH, DH)],
                wq_buf.at[slot, g, rows],
                wq_sem.at[slot],
            ).start(priority=j)

    def start_wo(br, u, i):
        slot = _slot(_group(u))
        for j in range(2):
            g = 2 * i + j
            pltpu.make_async_copy(
                wo_hbm[br].at[_rows(_head(u, g) * DH + _batch(u) * WO_ROWS, WO_ROWS)],
                wo_buf.at[slot, _rows(g * DH + _batch(u) * WO_ROWS, WO_ROWS)],
                wo_sem.at[slot],
            ).start(priority=j)

    def start_x(br, i):
        rows = _rows((i >> 2) * X_ROWS, X_ROWS)
        for j in range(2):
            b = (i & 3) + 4 * j
            pltpu.make_async_copy(
                x_hbm[br].at[b, rows], x_buf.at[br, b, rows], x_sem.at[br]
            ).start(priority=j)

    def start_out(batches):
        pieces = [(b, pl.ds(r, OUT_ROWS)) for r in range(0, SQ, OUT_ROWS) for b in batches]
        for i, idx in enumerate(pieces):
            pltpu.make_async_copy(res.at[idx], out_hbm.at[idx], out_sem).start(priority=i % 2)

    def wait_kv(u):
        for j, buf in enumerate((k_buf, v_buf)):
            _wait_filled(buf.at[_slot(u)], kv_sem.at[j, _slot(u)])

    def wait_weights(buf, sem, u):
        _wait_filled(buf.at[_slot(_group(u))], sem.at[_slot(_group(u))])

    def q_proj(u, after_tile):
        w = []
        for t in range(TILES):
            w.append(jnp.concatenate(
                [wq_buf[_slot(_group(u)), g, t * 128:(t + 1) * 128] for g in range(G)], axis=1))
            after_tile(t)
        q = jnp.dot(x_buf[_branch(u), _batch(u)], jnp.concatenate(w, axis=0),
                    preferred_element_type=F32)
        q = (q * Q_SCALE).astype(BF16)
        for g in range(G):
            q_buf[u & (2 * B - 1), g] = q[:, g * DH:(g + 1) * DH]

    def unit(u, starts, branches):
        started = dict(c=0, q=0, o=0)
        streams = dict(c=(start_kv, u + AHEAD),
                       q=(start_wq, u + AHEAD + 2 * B),
                       o=(start_wo, u + AHEAD + B))

        def start(kinds):
            for kind in kinds:
                fn, target = streams[kind]
                i = started[kind]
                if kind == "c":
                    which = ((K_ORDER[i], V_ORDER[i]),)
                elif kind == "q":
                    which = (i % 2, WQ_PARTS[i // 2])
                else:
                    which = (i,)
                for br in branches:
                    pl.when(_branch(target) == br)(lambda: fn(br, target, *which))
                started[kind] += 1

        probs = []
        for g in range(G):
            s = lax.dot_general(q_buf[u & (2 * B - 1), g], k_buf[_slot(u), g],
                                (((1,), (1,)), ((), ())), preferred_element_type=F32)
            p = jnp.exp2(s - jnp.max(s, axis=-1, keepdims=True))
            probs.append((p.astype(BF16), 1.0 / jnp.sum(p, axis=-1, keepdims=True)))
            start(starts["qk"][g])
        if "q_proj" in starts:
            q_proj(u + B, lambda t: start(starts["q_proj"][t]))
        heads = []
        for g, (p, inv_sum) in enumerate(probs):
            o = jnp.dot(p, v_buf[_slot(u), g], preferred_element_type=F32)
            heads.append((o * inv_sum).astype(BF16))
            start(starts["pv"][g])
        w = []
        for t in range(TILES):
            w.append(wo_buf[_slot(_group(u)), :, t * 128:(t + 1) * 128])
            start(starts["out_proj"][t])
        assert started["c"] == KV_PAIRS
        assert (started["q"], started["o"]) in ((0, 0), (WQ_PAIRS, WO_PAIRS))
        return acc[_branch(u), _batch(u)] + jnp.dot(
            jnp.concatenate(heads, axis=1), jnp.concatenate(w, axis=1),
            preferred_element_type=F32)

    assert (AHEAD, KV_PAIRS, G, WO_PAIRS) == (3, 2 * B, 4, 2)

    @pl.loop(0, X_PAIRS)
    def _(i):
        start_x(0, i)

    @pl.loop(0, B)
    def _(b):
        for i in range(2):
            start_wq(0, b, i)

    @pl.loop(0, B)
    def _(b):
        for i in range(2):
            start_kv(0, 0, (2 * b + i,) * 2)
            start_wo(0, b, i)
            start_wq(0, B + b, i)
            acc[i, b] = jnp.zeros((SQ, D), F32)

    for i in range(2):
        start_wq(0, 2 * B, i)
        start_wo(0, B, i)

    _wait_filled(x_buf.at[0], x_sem.at[0])
    wait_weights(wq_buf, wq_sem, 0)

    @pl.loop(0, B)
    def _(b):
        u, i = 1 + (b >> 2), b & 3
        for g in range(G):
            start_kv(0, u, (G * i + g,) * 2)
        pl.when(i < 2)(lambda: start_wo(0, u + B, i))
        pl.when(i >= 2)(lambda: start_wq(0, u + 2 * B, i - 2))
        q_proj(b, lambda t: None)

    @pl.loop(0, UNITS - B)
    def _(u):
        @pl.when(_batch(u) == 0)
        def _():
            wait_weights(wo_buf, wo_sem, u)
            wait_weights(wq_buf, wq_sem, u + B)

        wait_kv(u)
        pl.when(u == UNITS_PER_BRANCH - B)(lambda: _wait_filled(x_buf.at[1], x_sem.at[1]))
        pl.when(u < X_PAIRS)(lambda: start_x(1, u))
        acc[_branch(u), _batch(u)] = unit(u, MAIN_STARTS, (0, 1))

    wait_weights(wo_buf, wo_sem, UNITS - B)

    @pl.loop(0, B)
    def _(b):
        u = UNITS - B + b
        wait_kv(u)
        res[b, :, :D] = acc[0, b].astype(BF16)
        pl.when(b == B - 2)(lambda: start_out(range(B - 2)))
        res[b, :, D:] = unit(u, LAST_GROUP_STARTS, (1,)).astype(BF16)
        pl.when(b == B - 2)(lambda: start_out([B - 2]))

    start_out([B - 1])


def _kernel(ax, ak, av, awq, awo, bx, bk, bv, bwq, bwo, out_hbm, *scratch):
    res, out_sem = scratch[-2:]
    pl.run_scoped(
        lambda *sems: _pipeline((ax, bx), (ak, bk), (av, bv), (awq, bwq), (awo, bwo),
                                out_hbm, *scratch, *sems),
        pltpu.SemaphoreType.DMA((2, SLOTS)),
        pltpu.SemaphoreType.DMA((SLOTS,)),
        pltpu.SemaphoreType.DMA((SLOTS,)),
        pltpu.SemaphoreType.DMA((2,)),
    )
    pltpu.make_async_copy(res, out_hbm, out_sem).wait()


@jax.jit
def pallas_concat_heads__gqa_block_cached__mha_block_cached__near_ridge_kernel(
    A_x: jax.Array,
    A_k_cache: jax.Array,
    A_v_cache: jax.Array,
    A_wq: jax.Array,
    A_wo: jax.Array,
    B_x: jax.Array,
    B_k_cache: jax.Array,
    B_v_cache: jax.Array,
    B_wq: jax.Array,
    B_wo: jax.Array,
):
    args = (A_x, A_k_cache, A_v_cache, A_wq, A_wo, B_x, B_k_cache, B_v_cache, B_wq, B_wo)
    shapes = ((B, SQ, D), (B, H, SK, DH), (B, H, SK, DH), (D, H * DH), (H * DH, D)) * 2
    assert all(a.shape == s and a.dtype == BF16 for a, s in zip(args, shapes))

    return pl.pallas_call(
        _kernel,
        out_shape=jax.ShapeDtypeStruct((B, SQ, 2 * D), BF16),
        in_specs=[pl.BlockSpec(memory_space=pl.ANY)] * len(args),
        out_specs=pl.BlockSpec(memory_space=pl.ANY),
        scratch_shapes=[
            pltpu.VMEM((2, B, SQ, D), BF16),
            pltpu.VMEM((SLOTS, G, SK, DH), BF16),
            pltpu.VMEM((SLOTS, G, SK, DH), BF16),
            pltpu.VMEM((SLOTS, G, D, DH), BF16),
            pltpu.VMEM((SLOTS, G * DH, D), BF16),
            pltpu.VMEM((2 * B, G, SQ, DH), BF16),
            pltpu.VMEM((2, B, SQ, D), F32),
            pltpu.VMEM((B, SQ, 2 * D), BF16),
            pltpu.SemaphoreType.DMA(()),
        ],
        compiler_params=pltpu.CompilerParams(
            vmem_limit_bytes=64 * 1024 * 1024,
            disable_bounds_checks=True,
        ),
    )(*args)
```
